```python
import jax
import jax.numpy as jnp

def _softmax(x, axis=-1):
    return jax.nn.softmax(x, axis=axis)

def _gelu(x):
    return jax.nn.gelu(x, approximate=True)

def _silu(x):
    return jax.nn.silu(x)

def _sigmoid(x):
    return jax.nn.sigmoid(x)

def _layernorm(x, axis=-1, eps=1e-05):
    m = jnp.mean(x, axis=axis, keepdims=True)
    v = jnp.var(x, axis=axis, keepdims=True)
    return (x - m) / jnp.sqrt(v + eps)

def _scatter_add(tgt, idx, src, axis=0):
    return tgt.at[idx].add(src)

def _segment_sum(src, seg, n):
    return jax.ops.segment_sum(src, seg, n)

class _Rng:

    def __init__(self, key):
        self._k = key

    def _next(self):
        self._k, sub = jax.random.split(self._k)
        return sub

    def normal(self, shape):
        return jax.random.normal(self._next(), shape, dtype=jnp.bfloat16)

    def randint(self, lo, hi, shape):
        return jax.random.randint(self._next(), shape, lo, hi, dtype=jnp.int32)

    def uniform(self, shape, lo=0.0, hi=1.0):
        return jax.random.uniform(self._next(), shape, jnp.bfloat16, lo, hi)

    def permutation(self, n):
        return jax.random.permutation(self._next(), n)
kernel_name = 'interleave_layers__linear_kernel_hedgehog__mixer_gmlp__prompt'

def _fwd_setup_inputs():
    _rng = _Rng(jax.random.key(int.from_bytes(__import__("os").urandom(4), "little")))
    _w = lambda a: (lambda t: t.astype(jnp.bfloat16) if jnp.issubdtype(t.dtype, jnp.floating) else t)(jnp.asarray(a))

    def _A_setup():
        B, S, D, H = (1, 2048, 640, 32)
        Dh = D // H
        return {'x': _w((lambda *s: _rng.normal(s) * 0.05)(B, S, D)), 'wqkv': _w((lambda *s: _rng.normal(s) * 0.05)(D, 3 * D)), 'w_phi': _w((lambda *s: _rng.normal(s) * 0.05)(H, Dh, Dh) * Dh ** (-0.5)), 'wo': _w((lambda *s: _rng.normal(s) * 0.05)(D, D))}
    _A_in = _A_setup()

    def _B_setup():
        B, S, D, F = (1, 2048, 640, 1536)
        Fh = F // 2
        return {'x': _w((lambda *s: _rng.normal(s) * 0.05)(B, S, D)), 'w_in': _w((lambda *s: _rng.normal(s) * 0.05)(D, 2 * Fh)), 'w_sp': _w(0.01 * (lambda *s: _rng.normal(s) * 0.05)(S, S)), 'b_sp': _w(1.0 + 0.01 * (lambda *s: _rng.normal(s) * 0.05)(S)), 'w_out': _w((lambda *s: _rng.normal(s) * 0.05)(Fh, D))}
    _B_in = _B_setup()
    return {'A_x': _A_in['x'], 'A_wqkv': _A_in['wqkv'], 'A_w_phi': _A_in['w_phi'], 'A_wo': _A_in['wo'], 'B_x': _B_in['x'], 'B_w_in': _B_in['w_in'], 'B_w_sp': _B_in['w_sp'], 'B_b_sp': _B_in['b_sp'], 'B_w_out': _B_in['w_out']}

def _fwd_reference(A_x, A_wqkv, A_w_phi, A_wo, B_x, B_w_in, B_w_sp, B_b_sp, B_w_out):

    def _A_ref(x, wqkv, w_phi, wo):
        B, S, D = x.shape
        H = 32
        Dh = D // H
        qkv = (lambda x, *d: x.transpose(*d))((x @ wqkv).reshape(B, S, 3, H, Dh), 2, 0, 3, 1, 4)
        q, k, v = (qkv[0], qkv[1], qkv[2])
        pq = jnp.einsum('bhsd,hdf->bhsf', q, w_phi)
        pk = jnp.einsum('bhsd,hdf->bhsf', k, w_phi)
        phi_q = jnp.concatenate([_softmax(pq, axis=-1), _softmax(-pq, axis=-1)], axis=-1)
        phi_k = jnp.concatenate([_softmax(pk, axis=-1), _softmax(-pk, axis=-1)], axis=-1)
        kv = jnp.einsum('bhsf,bhsd->bhfd', phi_k, v)
        z = jnp.einsum('bhsf->bhf', phi_k)
        num = jnp.einsum('bhqf,bhfd->bhqd', phi_q, kv)
        den = jnp.einsum('bhqf,bhf->bhq', phi_q, z)[..., None] + 1e-06
        o = num / den
        return (lambda x, *d: x.transpose(*d))(o, 0, 2, 1, 3).reshape(B, S, D) @ wo

    def _B_ref(x, w_in, w_sp, b_sp, w_out):
        B, S, D = x.shape
        F = w_in.shape[-1]
        Fh = F // 2
        z = _gelu(jnp.einsum('bsd,df->bsf', x, w_in))
        z1 = z[..., :Fh].copy()
        z2 = _layernorm(z[..., Fh:], axis=-1)
        g = jnp.einsum('ts,bsf->btf', w_sp, z2) + b_sp[None, :, None]
        return jnp.einsum('bsf,fd->bsd', z1 * g, w_out)
    x = A_x
    x = x + _A_ref(_layernorm(x, axis=-1), A_wqkv, A_w_phi, A_wo)
    x = x + _B_ref(_layernorm(x, axis=-1), B_w_in, B_w_sp, B_b_sp, B_w_out)
    x = x + _A_ref(_layernorm(x, axis=-1), A_wqkv, A_w_phi, A_wo)
    x = x + _B_ref(_layernorm(x, axis=-1), B_w_in, B_w_sp, B_b_sp, B_w_out)
    return x

def setup_inputs():
    _inp = _fwd_setup_inputs()
    _gk = jax.random.fold_in(jax.random.key(int.from_bytes(__import__("os").urandom(4), "little")), 2 ** 31 - 1)
    _shapes = [[1, 2048, 640]]
    _dtypes = ['bfloat16']
    _gks = jax.random.split(_gk, len(_shapes))
    _gs = [jax.random.normal(k, s, dtype=jnp.dtype(d)) * 0.05 for k, s, d in zip(_gks, _shapes, _dtypes)]
    _inp['grad_out'] = _gs[0]
    return _inp

def reference(A_x, A_wqkv, A_w_phi, A_wo, B_w_in, B_w_sp, B_b_sp, B_w_out, B_x, grad_out):
    _const = dict(B_x=B_x)

    def _f(*_d):
        return _fwd_reference(**{'A_x': _d[0], 'A_wqkv': _d[1], 'A_w_phi': _d[2], 'A_wo': _d[3], 'B_w_in': _d[4], 'B_w_sp': _d[5], 'B_b_sp': _d[6], 'B_w_out': _d[7], **_const})
    _out, _vjp = jax.vjp(_f, A_x, A_wqkv, A_w_phi, A_wo, B_w_in, B_w_sp, B_b_sp, B_w_out)
    _grads = _vjp(grad_out)
    _out0 = jnp.asarray(_out)
    return (_out0, *[jnp.asarray(_g) for _g in _grads])
```

```python
import numpy as np

import jax
import jax.numpy as jnp
from jax import lax
import jax.experimental.pallas as pl
import jax.experimental.pallas.tpu as pltpu

S, D, H, DH, FH = 2048, 640, 32, 20, 768
NG = 16
GR = 40
CH = dict(attn1=512, attn2_mlp1=512, mlp2=256, mlp2_b=512, mlp1_attn2_b=512, attn1_b=512)
F32, BF16 = jnp.float32, jnp.bfloat16
EPS = 1e-5
GC = float(np.sqrt(2.0 / np.pi))
GA = 0.044715

_r = np.arange(D)
_HEAD_R = (_r // GR) * 2 + _r % 2
_FEAT_R = ((_r % GR) // 8) * 4 + (_r % 8) // 2
_COLV = np.stack([_r // DH, _r % DH] + [0 * _r] * 126, 1).astype(np.int32)
_ROWV = np.stack([_HEAD_R, _FEAT_R] + [0 * _r] * 6, 0).astype(np.int32)

NN = (((1,), (0,)), ((), ()))
NT = (((1,), (1,)), ((), ()))


def _dot(a, b, dims=NN):
    return lax.dot_general(a, b, dims, preferred_element_type=F32)


def _ln_fwd(x):
    n = x.shape[0]
    xc = x - jnp.sum(x, axis=0, keepdims=True) * (1.0 / n)
    rstd = lax.rsqrt(jnp.sum(xc * xc, axis=0, keepdims=True) * (1.0 / n) + EPS)
    return xc * rstd, rstd


def _ln_bwd(dy, xh, rstd):
    n = dy.shape[0]
    m1 = jnp.sum(dy, axis=0, keepdims=True) * (1.0 / n)
    m2 = jnp.sum(dy * xh, axis=0, keepdims=True) * (1.0 / n)
    return (dy - m1 - xh * m2) * rstd


def _gelu(u):
    t = jnp.tanh(GC * (u + GA * u * u * u))
    return 0.5 * u * (1.0 + t)


def _gelu_both(u):
    u2 = u * u
    t = jnp.tanh(u * (GC + (GC * GA) * u2))
    h = 0.5 * (1.0 + t)
    return u * h, h + u * (1.0 - t * t) * (0.5 * GC + (1.5 * GC * GA) * u2)


def _head_reduce(rows, op):
    r = rows[0]
    for x in rows[1:]:
        r = op(r, x)
    r = op(r, pltpu.roll(r, 4, 0))
    return op(r, pltpu.roll(r, 2, 0))


def _rows(p):
    return [p[8 * i:8 * i + 8] for i in range(p.shape[0] // 8)]


def _feature_map(p):
    rows = _rows(p)
    mx = _head_reduce(rows, jnp.maximum)
    mn = _head_reduce(rows, jnp.minimum)
    ep = [jnp.exp(x - mx) for x in rows]
    en = [jnp.exp(mn - x) for x in rows]
    rp = 1.0 / _head_reduce(ep, jnp.add)
    rn = 1.0 / _head_reduce(en, jnp.add)
    return jnp.concatenate([e * rp for e in ep] + [e * rn for e in en], 0)


def _feature_map_bwd(phi, dphi):
    t = _rows(phi * dphi)
    ph = _rows(phi)
    sp = _head_reduce(t[:5], jnp.add)
    sn = _head_reduce(t[5:], jnp.add)
    return jnp.concatenate(
        [(t[i] - t[5 + i]) - (ph[i] * sp - ph[5 + i] * sn) for i in range(5)], 0)


def _band(j):
    return max(j - 1, 0) * 128, min(j + 2, 5) * 128


def _kernel(x_hbm, wqkv_hbm, wphi_ref, wo_hbm, win_hbm, wsp_hbm, bsp_ref, wout_hbm, go_hbm,
            colv_ref, rowv_ref,
            out_hbm, dx_hbm, dwqkv_hbm, dwphi_ref, dwo_hbm, dwin_hbm, dwsp_hbm, dbsp_ref,
            dwout_hbm, stash_hbm,
            STG0, STG1, X, bOO, bPH, bVA, bXA, bXB, bUU, bGG, bMM, Z2N, DGN, DGT, DQ, DY, DEN, RS, KVA, KVT, KVN,
            WSP, WQKV, WO, WEFF, WEFFT, WOP, WOPT, WIN, WINT, WOUT, WOUTT, PHI, PERM, WQKT,
            AQKV, AO, AIN, AOUT, ADB, WP, sems):
    PHQ, PHK, UU, VA = 0, 1280, 0, 0
    def copy(src, dst, i):
        return pltpu.make_async_copy(src, dst, sems.at[i])

    def chunk_loop(body, width, n=None):
        def step(c, carry):
            body(pl.ds(pl.multiple_of(c * width, 128), width))
            return carry
        lax.fori_loop(0, n or S // width, step, 0)

    ld_wqkv, ld_x, ld_wo = copy(wqkv_hbm, WQKV, 0), copy(x_hbm, STG0, 1), copy(wo_hbm, WO, 2)
    ld_win, ld_wout = copy(win_hbm, WIN, 3), copy(wout_hbm, WOUT, 4)
    ld_wsp, ld_go = copy(wsp_hbm, WSP, 5), copy(go_hbm, STG1, 6)
    for cp in (ld_wqkv, ld_wo, ld_x):
        cp.start()
    bufs = dict(o=bOO, q=bPH.at[0:1280], k=bPH.at[1280:2560], v=bVA, a=bXA,
                b=bXB, u=bUU, g=bGG, m=bMM)

    def park(names, out, start):
        off = 0
        for i, (n, v) in enumerate(bufs.items()):
            h = stash_hbm.at[off:off + v.shape[0]]
            off += v.shape[0]
            if n in names:
                cp = copy(v, h, 15 + i) if out else copy(h, v, 15 + i)
                cp.start() if start else cp.wait()

    hc, dc = colv_ref[:, 0:1], colv_ref[:, 1:2]
    hr, fr = rowv_ref[0:1, :], rowv_ref[1:2, :]
    same_head = hc == hr
    WP[...] = jnp.zeros_like(WP)
    for h in range(H):
        WP[h * DH:(h + 1) * DH, 0:DH] = wphi_ref[h].astype(F32)
    sel = (lax.broadcasted_iota(jnp.int32, (128, D), 0) == fr).astype(BF16)
    PHI[...] = jnp.where(same_head, _dot(WP[...].astype(BF16), sel), 0.0).astype(BF16)
    PERM[...] = jnp.where(same_head & (dc == fr), 1.0, 0.0).astype(BF16)

    ld_wqkv.wait()
    for part, mat in enumerate((PHI, PHI, PERM)):
        for j in range(5):
            lo, hi = _band(j)
            co = part * D + j * 128
            w = _dot(WQKV[:, part * D + lo:part * D + hi], mat[lo:hi, j * 128:(j + 1) * 128])
            WEFF[:, co:co + 128] = w.astype(BF16)
            WEFFT[co:co + 128, :] = w.T.astype(BF16)
    WQKT[...] = WQKV[:, 0:2 * D].T
    ld_wo.wait()
    permt = PERM[...].T
    for j in range(5):
        lo, hi = _band(j)
        w = _dot(permt[j * 128:(j + 1) * 128, lo:hi], WO[lo:hi, :])
        WOP[j * 128:(j + 1) * 128, :] = w.astype(BF16)
        WOPT[:, j * 128:(j + 1) * 128] = w.astype(BF16).T

    ld_x.wait()
    pair = (lax.broadcasted_iota(jnp.int32, (48, 128), 0) % 2
            == lax.broadcasted_iota(jnp.int32, (48, 128), 1) % 2)

    def finish_kv(slot):
        for g in range(NG):
            kv = jnp.where(pair, KVA[g], 0.0)
            KVT[slot, g] = kv.astype(BF16)
            kvt = jnp.concatenate([kv, jnp.zeros((80, 128), F32)], 0).T
            KVN[slot, g] = kvt[0:80].astype(BF16)

    def rows8(v):
        return jnp.broadcast_to(v, (8, v.shape[1]))

    def accum(ref, idx, val, first):
        ref[idx] = val if first else ref[idx] + val

    def fwd_layer(l):
        KVA[...] = jnp.zeros_like(KVA)
        if l == 0:
            for cp in (ld_win, ld_wout, ld_wsp, ld_go):
                cp.start()

        def attn0(s):
            if l == 0:
                x = STG0[s, :].T.astype(F32)
                X[:, s] = x
            else:
                x = X[:, s]
            xn, rstd = _ln_fwd(x)
            bXA[:, s] = xn.astype(BF16)
            RS[l, 0, :, s] = rows8(rstd)
            return xn.astype(BF16)

        def attn1(s, xn):
            ones = jnp.ones((8, xn.shape[1]), F32)
            for q in range(4):
                r0 = q * 160
                pk = _dot(WEFFT[D + r0:D + r0 + 160, :], xn)
                v = _dot(WEFFT[2 * D + r0:2 * D + r0 + 160, :], xn)
                pq = _dot(WEFFT[r0:r0 + 160, :], xn)
                for i in range(4):
                    g = q * 4 + i
                    sl = slice(i * GR, (i + 1) * GR)
                    phk = _feature_map(pk[sl]).astype(BF16)
                    va = jnp.concatenate([v[sl], ones], 0).astype(BF16)
                    bPH[PHK + g * 80:PHK + g * 80 + 80, s] = phk
                    bVA[VA + g * 48:VA + g * 48 + 48, s] = va
                    KVA[g, :, 0:80] += _dot(va, phk, NT)
                    bPH[PHQ + g * 80:PHQ + g * 80 + 80, s] = _feature_map(pq[sl]).astype(BF16)
        with jax.named_scope("attn1"):
            chunk_loop(lambda s: attn1(s, attn0(s)), CH['attn1'])
        finish_kv(l)
        if l == 0:
            ld_win.wait()
            WINT[...] = WIN[...].T
            ld_wout.wait()
            WOUTT[...] = WOUT[...].T
        else:
            park('bugm', True, False)

        def attn2(s):
            outs = []
            for g in range(NG):
                num = _dot(KVT[l, g, :, 0:80], bPH[PHQ + g * 80:PHQ + g * 80 + 80, s])
                rden = 1.0 / (num[40:48] + 1e-6)
                DEN[l, g * 8:g * 8 + 8, s] = rden
                outs += [num[8 * i:8 * i + 8] * rden for i in range(5)]
            o = jnp.concatenate(outs, 0).astype(BF16)
            bOO[:, s] = o
            x = X[:, s] + _dot(WOPT[...], o)
            X[:, s] = x
            xn, rstd = _ln_fwd(x)
            bXB[:, s] = xn.astype(BF16)
            RS[l, 1, :, s] = rows8(rstd)
            return xn.astype(BF16)

        def mlp1(s, xn):
            u2 = _dot(WINT[FH:2 * FH, :], xn)
            bUU[UU + FH:UU + 2 * FH, s] = u2.astype(BF16)
            z2n, rstd2 = _ln_fwd(_gelu(u2))
            bUU[UU:UU + FH, s] = _dot(WINT[0:FH, :], xn).astype(BF16)
            Z2N[l, :, s] = z2n.astype(BF16)
            RS[l, 2, :, s] = rows8(rstd2)
        with jax.named_scope("attn2_mlp1"):
            chunk_loop(lambda s: mlp1(s, attn2(s)), CH['attn2_mlp1'])
        if l == 0:
            park('oqkva', True, True)
            ld_wsp.wait()

            def mlp2(s):
                z1 = _gelu(bUU[UU:UU + FH, s].astype(F32))
                g = _dot(Z2N[l], WSP[s, :], NT) + bsp_ref[:, s].astype(F32)
                bGG[:, s] = g.astype(BF16)
                m = (z1 * g).astype(BF16)
                bMM[:, s] = m
                X[:, s] += _dot(WOUTT[...], m)
            with jax.named_scope("mlp2"):
                chunk_loop(mlp2, CH['mlp2'])
            park('oqkva', True, False)
            park('bugm', True, True)

    fwd_layer(0)
    fwd_layer(1)
    ld_go.wait()
    wr_out = copy(STG0, out_hbm, 9)

    def wgrad(acc, final, lhs, rhs, n, l):
        def body(t):
            d = _dot(lhs[...], rhs[t, :], NT)
            if l == 1:
                acc[:, t] = d
            else:
                final[:, t] = (acc[:, t] + d).astype(BF16)
        chunk_loop(body, n, acc.shape[1] // n)

    def bwd_layer(l):
        if l == 0:
            park('bugm', False, False)
            park('oq', False, True)

        def mlp2_b(s):
            z1, gp = _gelu_both(bUU[UU:UU + FH, s].astype(F32))
            if l == 1:
                dy = STG1[s, :].T
                dm = _dot(WOUT[...], dy)
                g = _dot(Z2N[l], WSP[s, :], NT) + bsp_ref[:, s].astype(F32)
                m = (z1 * g).astype(BF16)
                bMM[:, s] = m
                y = _dot(WOUTT[...], m)
            else:
                dy = X[:, s].astype(BF16)
                dm = _dot(WOUT[...], dy)
                g = bGG[:, s].astype(F32)
            DY[:, s] = dy
            dg = dm * z1
            accum(ADB, (slice(None), s), jnp.sum(dg, axis=0, keepdims=True), l == 1)
            dg = dg.astype(BF16)
            DGT[:, s] = dg
            DGN[s, l * FH:(l + 1) * FH] = dg.T
            bUU[UU:UU + FH, s] = (dm * g * gp).astype(BF16)
            if l == 1:
                STG0[s, :] = (X[:, s] + y).astype(BF16).T
                X[:, s] = dy.astype(F32)
        with jax.named_scope("mlp2_b"):
            chunk_loop(mlp2_b, CH['mlp2_b'])
        if l == 1:
            wr_out.start()
        with jax.named_scope("dwout"):
            wgrad(AOUT, WOUT, bMM, DY, 128, l)
        KVA[...] = jnp.zeros_like(KVA)
        if l == 0:
            wr.append(copy(WOUT, dwout_hbm, 12))
            wr[-1].start()
            park('oq', False, False)
            park('kva', False, True)

        def mlp1_b(s):
            _, gp = _gelu_both(bUU[UU + FH:UU + 2 * FH, s].astype(F32))
            dzn = _dot(DGT[...], WSP[:, s])
            dxn = _dot(WIN[:, 0:FH], bUU[UU:UU + FH, s])
            dz = _ln_bwd(dzn, Z2N[l, :, s].astype(F32), RS[l, 2, 0:1, s])
            du2 = (dz * gp).astype(BF16)
            bUU[UU + FH:UU + 2 * FH, s] = du2
            dxn = dxn + _dot(WIN[:, FH:2 * FH], du2)
            return dxn

        def attn2_b(s, dxn):
            dx = X[:, s] + _ln_bwd(dxn, bXB[:, s].astype(F32), RS[l, 1, 0:1, s])
            X[:, s] = dx
            dy = dx.astype(BF16)
            DY[:, s] = dy
            do = _dot(WOP[...], dy)
            o = bOO[:, s].astype(F32)
            for g in range(NG):
                dn = do[g * GR:(g + 1) * GR] * jnp.concatenate([DEN[l, g * 8:g * 8 + 8, s]] * 5, 0)
                t = _rows(dn * o[g * GR:(g + 1) * GR])
                dd = -(t[0] + t[1] + t[2] + t[3] + t[4])
                dna = jnp.concatenate([dn, dd], 0).astype(BF16)
                phq = bPH[PHQ + g * 80:PHQ + g * 80 + 80, s]
                KVA[g, :, 0:80] += _dot(dna, phq, NT)
                dphi = _dot(KVN[l, g, :, 0:48], dna)
                DQ[g * GR:(g + 1) * GR, s] = _feature_map_bwd(phq.astype(F32), dphi)
            r = pl.ds(pl.multiple_of(s.start // 512 * 160, 32), 160)
            accum(AIN, (r, slice(0, FH)), _dot(bXB[r, :], bUU[0:FH, :], NT), l == 1)
        with jax.named_scope("mlp1_attn2_b"):
            chunk_loop(lambda s: attn2_b(s, mlp1_b(s)), CH['mlp1_attn2_b'])
        finish_kv(2)
        with jax.named_scope("dwin"):
            wgrad(AIN.at[:, FH:2 * FH], WIN.at[:, FH:2 * FH], bXB, bUU.at[FH:2 * FH], 256, l)
            if l == 0:
                WIN[:, 0:FH] = AIN[:, 0:FH].astype(BF16)
        if l == 1:
            park('bugm', False, True)
        else:
            wr.append(copy(WIN, dwin_hbm, 11))
            wr[-1].start()
        with jax.named_scope("dwo"):
            wgrad(AO, WOP, bOO, DY, 128, l)
        if l == 0:
            park('kva', False, False)

        def attn1_b(s):
            dks, dvs = [], []
            for g in range(NG):
                phk = bPH[PHK + g * 80:PHK + g * 80 + 80, s]
                dphi = _dot(KVN[2, g, :, 0:48], bVA[VA + g * 48:VA + g * 48 + 48, s])
                dks.append(_feature_map_bwd(phk.astype(F32), dphi))
                dvs.append(_dot(KVT[2, g, :, 0:80], phk)[0:GR])
            d = [jnp.concatenate(t, 0).astype(BF16) for t in ([DQ[:, s]], dks, dvs)]
            for i in range(3):
                bPH[i * D:(i + 1) * D, s] = d[i]
            return d

        def attn0_b(s, d):
            dxn = (_dot(WEFF[:, 0:D], d[0]) + _dot(WEFF[:, 2 * D:3 * D], d[2])) + _dot(WEFF[:, D:2 * D], d[1])
            dx = X[:, s] + _ln_bwd(dxn, bXA[:, s].astype(F32), RS[l, 0, 0:1, s])
            if l == 1:
                X[:, s] = dx
            else:
                STG1[s, :] = dx.astype(BF16).T
        with jax.named_scope("attn1_b"):
            chunk_loop(lambda s: attn0_b(s, attn1_b(s)), CH['attn1_b'])
        if l == 0:
            wr.append(copy(STG1, dx_hbm, 10))
            wr[-1].start()
        with jax.named_scope("dwqkv"):
            wgrad(AQKV, WEFF, bXA, bPH.at[PHQ:PHQ + 3 * D], 384, l)

    wr = []
    bwd_layer(1)
    bwd_layer(0)

    dbsp_ref[...] = ADB[...].astype(BF16)
    for j in range(5):
        lo, hi = _band(j)
        t = slice(j * 128, (j + 1) * 128)
        WO[t, :] = _dot(PERM[t, lo:hi], WOP[lo:hi, :]).astype(BF16)
    wr.append(copy(WO, dwo_hbm, 13))
    wr[-1].start()
    for part, mat in enumerate((PHI, PHI, PERM)):
        for j in range(5):
            lo, hi = _band(j)
            co = part * D + j * 128
            WQKV[:, co:co + 128] = _dot(WEFF[:, part * D + lo:part * D + hi],
                                        mat[j * 128:(j + 1) * 128, lo:hi], NT).astype(BF16)
    wr.append(copy(WQKV, dwqkv_hbm, 14))
    wr[-1].start()
    selt = sel.astype(F32).T.astype(BF16)
    dphis = []
    for j in range(5):
        lo, hi = _band(j)
        t = slice(j * 128, (j + 1) * 128)
        d = (_dot(WQKT[t, :], WEFF[:, lo:hi])
             + _dot(WQKT[D + j * 128:D + (j + 1) * 128, :], WEFF[:, D + lo:D + hi]))
        d = jnp.where(same_head[t, lo:hi], d, 0.0).astype(BF16)
        dphis.append(_dot(d, selt[lo:hi]))
    dphi = jnp.concatenate(dphis, 0)
    for h in range(H):
        dwphi_ref[h] = dphi[h * DH:(h + 1) * DH, 0:DH].astype(BF16)

    def dwsp(s):
        WSP[s, :] = (_dot(DGN[s, 0:FH], Z2N[0]) + _dot(DGN[s, FH:2 * FH], Z2N[1])).astype(BF16)
        copy(WSP.at[s], dwsp_hbm.at[s], 5).start()
    dwsp(pl.ds(S - 256, 256))
    with jax.named_scope("dwsp"):
        chunk_loop(dwsp, 256, 7)
    ld_wsp.wait()
    wr_out.wait()
    for cp in wr:
        cp.wait()


@jax.jit
def pallas_interleave_layers__linear_kernel_hedgehog__mixer_gmlp__prompt_kernel(
    A_x: jax.Array,
    A_wqkv: jax.Array,
    A_w_phi: jax.Array,
    A_wo: jax.Array,
    B_x: jax.Array,
    B_w_in: jax.Array,
    B_w_sp: jax.Array,
    B_b_sp: jax.Array,
    B_w_out: jax.Array,
    grad_out: jax.Array,
):
    del B_x
    hbm = pl.BlockSpec(memory_space=pl.ANY)
    vmem = pl.BlockSpec(memory_space=pltpu.VMEM)
    bf = lambda *s: pltpu.VMEM(s, BF16)
    f32 = lambda *s: pltpu.VMEM(s, F32)
    sds = lambda *s: jax.ShapeDtypeStruct(s, BF16)
    outs = pl.pallas_call(
        _kernel,
        out_shape=(sds(S, D), sds(S, D), sds(D, 3 * D), sds(H, DH, DH), sds(D, D),
                   sds(D, 2 * FH), sds(S, S), sds(1, S), sds(FH, D), sds(8320, S)),
        in_specs=[hbm, hbm, vmem, hbm, hbm, hbm, vmem, hbm, hbm, vmem, vmem],
        out_specs=(hbm, hbm, hbm, vmem, hbm, hbm, hbm, vmem, hbm, hbm),
        scratch_shapes=[
            bf(S, D), bf(S, D), f32(D, S), bf(D, S), bf(4 * D, S), bf(768, S), bf(D, S), bf(D, S), bf(2 * FH, S), bf(FH, S), bf(FH, S),
            bf(2, FH, S), bf(S, 2 * FH), bf(FH, S),
            f32(D, S), bf(D, S), f32(2, 128, S), f32(2, 3, 8, S),
            f32(NG, 48, 128), bf(3, NG, 48, 128), bf(3, NG, 80, 128),
            bf(S, S), bf(D, 3 * D), bf(D, D), bf(D, 3 * D), bf(3 * D, D), bf(D, D), bf(D, D),
            bf(D, 2 * FH), bf(2 * FH, D), bf(FH, D), bf(D, FH), bf(D, D), bf(D, D), bf(2 * D, D),
            f32(D, 3 * D), f32(D, D), f32(D, 2 * FH), f32(FH, D), f32(1, S), f32(D, 128),
            pltpu.SemaphoreType.DMA((24,)),
        ],
        compiler_params=pltpu.CompilerParams(vmem_limit_bytes=127 << 20),
    )(A_x.reshape(S, D), A_wqkv, A_w_phi, A_wo, B_w_in, B_w_sp, B_b_sp.reshape(1, S), B_w_out,
      grad_out.reshape(S, D), _COLV, _ROWV)
    out, dx, dwqkv, dwphi, dwo, dwin, dwsp, dbsp, dwout, _ = outs
    return (out.reshape(1, S, D), dx.reshape(1, S, D), dwqkv, dwphi, dwo, dwin, dwsp,
            dbsp.reshape(S), dwout)
```
